```python
import os as _os
_os.environ.setdefault("JAX_PLATFORMS", "cpu")
import jax
import jax.numpy as jnp

def _softmax(x, axis=-1):
    return jax.nn.softmax(x, axis=axis)
def _gelu(x):
    return jax.nn.gelu(x, approximate=True)
def _silu(x):
    return jax.nn.silu(x)
def _sigmoid(x):
    return jax.nn.sigmoid(x)
def _layernorm(x, axis=-1, eps=1e-5):
    m = jnp.mean(x, axis=axis, keepdims=True)
    v = jnp.var(x, axis=axis, keepdims=True)
    return (x - m) / jnp.sqrt(v + eps)
def _scatter_add(tgt, idx, src, axis=0):
    return tgt.at[idx].add(src)
def _segment_sum(src, seg, n):
    return jax.ops.segment_sum(src, seg, n)
class _Rng:
    def __init__(self, key):
        self._k = key
    def _next(self):
        self._k, sub = jax.random.split(self._k)
        return sub
    def normal(self, shape):
        return jax.random.normal(self._next(), shape, dtype=jnp.bfloat16)
    def randint(self, lo, hi, shape):
        return jax.random.randint(self._next(), shape, lo, hi, dtype=jnp.int32)
    def uniform(self, shape, lo=0.0, hi=1.0):
        return jax.random.uniform(self._next(), shape, jnp.bfloat16, lo, hi)
    def permutation(self, n):
        return jax.random.permutation(self._next(), n)


kernel_name = 'concat_heads__gqa_block_cached__sliding_block_cached__decode'

def setup_inputs():
    _rng = _Rng(jax.random.key(int.from_bytes(__import__("os").urandom(4), "little")))
    _w = (lambda a: (lambda t: t.astype(jnp.bfloat16) if jnp.issubdtype(t.dtype, jnp.floating) else t)(jnp.asarray(a)))
    def _A_setup():
        B, Sq, D = 2, 1, 448
        Hq, Hkv, Sk, Dh = 16, 8, 8192, 256
        assert Hq % Hkv == 0, (Hq, Hkv)
        return {
            "x": _w((lambda *s: _rng.normal(s) * 0.8)(B, Sq, D)),
            "k_cache": _w((lambda *s: _rng.normal(s) * 0.8)(B, Hkv, Sk, Dh)),
            "v_cache": _w((lambda *s: _rng.normal(s) * 0.05)(B, Hkv, Sk, Dh)),
            "wq": _w((lambda *s: _rng.normal(s) * 0.8)(D, Hq * Dh) * (D ** -0.5)),
            "wo": _w((lambda *s: _rng.normal(s) * 0.05)(Hq * Dh, D) * ((Hq * Dh) ** -0.5)),
        }
    _A_in = _A_setup()

    def _B_setup():
        B, Sq, D = 2, 1, 448
        Hq, Hkv, Sk, Dh = 16, 8, 8192, 256
        assert Hq % Hkv == 0, (Hq, Hkv)
        return {
            "x": _w((lambda *s: _rng.normal(s) * 0.8)(B, Sq, D)),
            "k_cache": _w((lambda *s: _rng.normal(s) * 0.8)(B, Hkv, Sk, Dh)),
            "v_cache": _w((lambda *s: _rng.normal(s) * 0.05)(B, Hkv, Sk, Dh)),
            "wq": _w((lambda *s: _rng.normal(s) * 0.8)(D, Hq * Dh) * (D ** -0.5)),
            "wo": _w((lambda *s: _rng.normal(s) * 0.05)(Hq * Dh, D) * ((Hq * Dh) ** -0.5)),
        }
    _B_in = _B_setup()

    return {
        "A_x": _A_in["x"],
        "A_k_cache": _A_in["k_cache"],
        "A_v_cache": _A_in["v_cache"],
        "A_wq": _A_in["wq"],
        "A_wo": _A_in["wo"],
        "B_x": _B_in["x"],
        "B_k_cache": _B_in["k_cache"],
        "B_v_cache": _B_in["v_cache"],
        "B_wq": _B_in["wq"],
        "B_wo": _B_in["wo"],
    }

def reference(A_x, A_k_cache, A_v_cache, A_wq, A_wo, B_x, B_k_cache, B_v_cache, B_wq, B_wo):
    def _A_ref(x, k_cache, v_cache, wq, wo):
        B, Sq, D = x.shape
        Hq, Dh = 16, 256
        Hkv = k_cache.shape[1]
        rep = Hq // Hkv
        q = (lambda x, *d: x.transpose(*d))((x @ wq).reshape(B, Sq, Hq, Dh), 0, 2, 1, 3)
        k = jnp.repeat(k_cache, rep, axis=1)
        v = jnp.repeat(v_cache, rep, axis=1)
        scores = jnp.einsum("bhqd,bhkd->bhqk", q, k) * (Dh ** -0.5)
        p = _softmax(scores, axis=-1)
        o = jnp.einsum("bhqk,bhkd->bhqd", p, v)
        return (lambda x, *d: x.transpose(*d))(o, 0, 2, 1, 3).reshape(B, Sq, Hq * Dh) @ wo

    def _B_ref(x, k_cache, v_cache, wq, wo):
        B, Sq, D = x.shape
        Hq, Dh = 16, 256
        Hkv, Sk = k_cache.shape[1], k_cache.shape[2]
        W = min(4096, max(256, Sk // 4))
        rep = Hq // Hkv
        q = (lambda x, *d: x.transpose(*d))((x @ wq).reshape(B, Sq, Hq, Dh), 0, 2, 1, 3)
        k = jnp.repeat(k_cache[:, :, Sk - W:, :], rep, axis=1)
        v = jnp.repeat(v_cache[:, :, Sk - W:, :], rep, axis=1)
        scores = jnp.einsum("bhqd,bhkd->bhqk", q, k) * (Dh ** -0.5)
        p = _softmax(scores, axis=-1)
        o = jnp.einsum("bhqk,bhkd->bhqd", p, v)
        return (lambda x, *d: x.transpose(*d))(o, 0, 2, 1, 3).reshape(B, Sq, Hq * Dh) @ wo

    a = _A_ref(A_x, A_k_cache, A_v_cache, A_wq, A_wo)
    b = _B_ref(B_x, B_k_cache, B_v_cache, B_wq, B_wo)
    return jnp.concatenate([a, b], axis=-1)
```

```python
import functools
import jax
import jax.numpy as jnp
from jax import lax
from jax.experimental import pallas as pl
from jax.experimental.pallas import tpu as pltpu

B, D, HQ, HKV, SK, DH = 2, 448, 16, 8, 8192, 256
W = 2048
E = HQ * DH
NT = (((1,), (1,)), ((), ()))
NN = (((1,), (0,)), ((), ()))
WG = 4
WR = D // WG


def build(CH=256, NB=4, SR=8, WC=512, wqb_at=8, compute=True):
    CA = SK // CH
    CB = W // CH
    NA = B * CA
    NJ = NA + B * CB
    NSL = E // WC

    def kernel(xa, xb, ak, av, awq, awo, bk, bv, bwq, bwo, o_hbm,
               kbuf, vbuf, wqbuf, wobuf, xbuf, q_scr, o_scr, m_scr, l_scr, acc_scr, out_scr,
               ksem, vsem, wqsem, wosem, xsem, osem):

        def decode(j, is_a):
            if is_a:
                return j // CA, j % CA, (j % CA) * CH
            jj = j - NA
            return jj // CB, jj % CB, (SK - W) + (jj % CB) * CH

        def issue(j, is_a):
            b, c, start = decode(j, is_a)
            slot = j % NB
            ks, vs = (ak, av) if is_a else (bk, bv)
            for s in range(0, CH, SR):
                st = start + s
                if not isinstance(st, int):
                    st = pl.multiple_of(st, SR)
                pltpu.make_async_copy(ks.at[b, :, pl.ds(st, SR), :], kbuf.at[slot, :, pl.ds(s, SR), :],
                                      ksem.at[slot]).start(priority=0)
                pltpu.make_async_copy(vs.at[b, :, pl.ds(st, SR), :], vbuf.at[slot, :, pl.ds(s, SR), :],
                                      vsem.at[slot]).start(priority=1)

        def issue_wq(br):
            w = (awq, bwq)[br]
            n = 0
            for i in range(WR // 8):
                for jc in range(E // 512 // 2):
                    for half in range(2):
                        c0 = (half * (E // 512 // 2) + jc) * 512
                        pltpu.make_async_copy(w.at[:, pl.ds(8 * i, 8), pl.ds(c0, 512)],
                                              wqbuf.at[br, :, pl.ds(8 * i, 8), pl.ds(c0, 512)],
                                              wqsem.at[br]).start(priority=half)

        def issue_wo(sl):
            for i in range(WR // 8):
                for br, w in enumerate((awo, bwo)):
                    pltpu.make_async_copy(w.at[:, pl.ds(8 * i, 8), pl.ds(sl * WC, WC)],
                                          wobuf.at[br, :, pl.ds(8 * i, 8), pl.ds(sl * WC, WC)],
                                          wosem.at[br * NSL + sl]).start(priority=br)

        def start_job(j):
            if isinstance(j, int):
                issue(j, j < NA)
            else:
                @pl.when(j < NA)
                def _():
                    issue(j, True)

                @pl.when(jnp.logical_and(j >= NA, j < NJ))
                def _():
                    issue(j, False)

                per = NSL // NB
                for t in range(NB):
                    @pl.when(j == NJ + t)
                    def _():
                        for sl in range(t * per, (t + 1) * per):
                            issue_wo(sl)

        xca = pltpu.make_async_copy(xa, xbuf.at[0], xsem.at[0])
        xcb = pltpu.make_async_copy(xb, xbuf.at[1], xsem.at[1])
        xca.start()
        issue_wq(0)
        for j in range(NB):
            start_job(j)
        xcb.start()

        q_scr[...] = jnp.zeros(q_scr.shape, q_scr.dtype)
        o_scr[...] = jnp.zeros(o_scr.shape, o_scr.dtype)

        def qproj(br):
            x2 = xbuf[br].astype(jnp.float32)
            rows = lax.broadcasted_iota(jnp.int32, (8, D), 0)
            x0 = jnp.broadcast_to(x2[0:1], (8, D))
            x1 = jnp.broadcast_to(x2[1:2], (8, D))
            xx = jnp.where(rows == 0, x0, jnp.where(rows == 1, x1, 0.0)).astype(jnp.bfloat16)
            w = wqbuf[br].reshape(D, E)
            q = lax.dot_general(xx, w, NN, preferred_element_type=jnp.float32)
            q = (q.astype(jnp.bfloat16).astype(jnp.float32) * (DH ** -0.5))
            for b in range(B):
                for h in range(HQ):
                    q_scr[br, b, h // 2, h:h + 1, :] = q[b:b + 1, h * DH:(h + 1) * DH]

        def wait_k(slot):
            pltpu.make_async_copy(kbuf.at[slot], kbuf.at[slot], ksem.at[slot]).wait()

        def wait_v(slot):
            pltpu.make_async_copy(vbuf.at[slot], vbuf.at[slot], vsem.at[slot]).wait()

        def job(j, br, is_a):
            b, c, start = decode(j, is_a)
            slot = j % NB
            C = CA if is_a else CB

            @pl.when(c == 0)
            def _():
                m_scr[...] = jnp.full(m_scr.shape, -jnp.inf, jnp.float32)
                l_scr[...] = jnp.zeros(l_scr.shape, jnp.float32)
                acc_scr[...] = jnp.zeros(acc_scr.shape, jnp.float32)

            wait_k(slot)
            if compute:
                s = None
                for g in range(HKV):
                    qg = q_scr[br, b, g].astype(jnp.bfloat16)
                    sg = lax.dot_general(qg, kbuf[slot, g], NT, preferred_element_type=jnp.float32)
                    s = sg if s is None else s + sg
                m_prev = m_scr[...]
                m_cur = jnp.max(s, axis=1, keepdims=True)
                m_new = jnp.maximum(m_prev, m_cur)
                alpha = jnp.exp(m_prev - m_new)
                p = jnp.exp(s - m_new[:, 0:1])
                l_scr[...] = alpha * l_scr[...] + jnp.sum(p, axis=1, keepdims=True)
                m_scr[...] = m_new
                pb = p.astype(jnp.bfloat16)
            wait_v(slot)
            if compute:
                grp = lax.broadcasted_iota(jnp.int32, (HQ, DH), 0) // 2
                acc = acc_scr[...] * alpha[:, 0:1]
                for g in range(HKV):
                    og = lax.dot_general(pb, vbuf[slot, g], NN, preferred_element_type=jnp.float32)
                    acc = acc + jnp.where(grp == g, og, 0.0)
                acc_scr[...] = acc
            start_job(j + NB)

            if is_a:
                @pl.when(j == wqb_at)
                def _():
                    issue_wq(1)

            if compute:
                @pl.when(c == C - 1)
                def _():
                    o = acc / l_scr[...][:, 0:1]
                    o = o.astype(jnp.bfloat16).astype(jnp.float32)
                    for h in range(HQ):
                        o_scr[br, pl.ds(b, 1), h * DH:(h + 1) * DH] = o[h:h + 1, :]

        xca.wait()
        pltpu.make_async_copy(wqbuf.at[0], wqbuf.at[0], wqsem.at[0]).wait()
        qproj(0)

        def body_a(j, carry):
            job(j, 0, True)
            return carry
        lax.fori_loop(0, NA, body_a, 0)

        xcb.wait()
        pltpu.make_async_copy(wqbuf.at[1], wqbuf.at[1], wqsem.at[1]).wait()
        qproj(1)

        def body_b(j, carry):
            job(j, 1, False)
            return carry
        lax.fori_loop(NA, NJ, body_b, 0)

        outs = [None, None]
        for sl in range(NSL):
            for br in range(2):
                dst = wobuf.at[br, :, :, pl.ds(sl * WC, WC)]
                pltpu.make_async_copy(dst, dst, wosem.at[br * NSL + sl]).wait()
                w = wobuf[br, :, :, sl * WC:(sl + 1) * WC].reshape(D, WC)
                ob = o_scr[br, :, sl * WC:(sl + 1) * WC].astype(jnp.bfloat16)
                part = lax.dot_general(ob, w, NT, preferred_element_type=jnp.float32)
                outs[br] = part if outs[br] is None else outs[br] + part
        out_scr[:, 0:D] = outs[0][0:B].astype(out_scr.dtype)
        out_scr[:, D:2 * D] = outs[1][0:B].astype(out_scr.dtype)
        oc = pltpu.make_async_copy(out_scr, o_hbm, osem.at[0])
        oc.start()
        oc.wait()

    @jax.jit
    def f(A_x, A_k_cache, A_v_cache, A_wq, A_wo, B_x, B_k_cache, B_v_cache, B_wq, B_wo):
        hbm = pl.BlockSpec(memory_space=pltpu.HBM)
        bf = jnp.bfloat16
        out = pl.pallas_call(
            kernel,
            out_shape=jax.ShapeDtypeStruct((B, 2 * D), bf),
            in_specs=[hbm] * 10,
            out_specs=hbm,
            scratch_shapes=[
                pltpu.VMEM((NB, HKV, CH, DH), bf),
                pltpu.VMEM((NB, HKV, CH, DH), bf),
                pltpu.VMEM((2, WG, WR, E), bf),
                pltpu.VMEM((2, WG, WR, E), bf),
                pltpu.VMEM((2, B, D), bf),
                pltpu.VMEM((2, B, HKV, HQ, DH), jnp.float32),
                pltpu.VMEM((2, 8, E), jnp.float32),
                pltpu.VMEM((HQ, 128), jnp.float32),
                pltpu.VMEM((HQ, 128), jnp.float32),
                pltpu.VMEM((HQ, DH), jnp.float32),
                pltpu.VMEM((B, 2 * D), bf),
                pltpu.SemaphoreType.DMA((NB,)),
                pltpu.SemaphoreType.DMA((NB,)),
                pltpu.SemaphoreType.DMA((2,)),
                pltpu.SemaphoreType.DMA((2 * NSL,)),
                pltpu.SemaphoreType.DMA((2,)),
                pltpu.SemaphoreType.DMA((1,)),
            ],
            compiler_params=pltpu.CompilerParams(vmem_limit_bytes=100 * 1024 * 1024),
        )(A_x.reshape(B, D), B_x.reshape(B, D), A_k_cache, A_v_cache,
          A_wq.reshape(WG, WR, E), A_wo.T.reshape(WG, WR, E),
          B_k_cache, B_v_cache,
          B_wq.reshape(WG, WR, E), B_wo.T.reshape(WG, WR, E))
        return out.reshape(B, 1, 2 * D)
    return f


_impl = build()


@jax.jit
def pallas_concat_heads__gqa_block_cached__sliding_block_cached__decode_kernel(
    A_x: jax.Array,
    A_k_cache: jax.Array,
    A_v_cache: jax.Array,
    A_wq: jax.Array,
    A_wo: jax.Array,
    B_x: jax.Array,
    B_k_cache: jax.Array,
    B_v_cache: jax.Array,
    B_wq: jax.Array,
    B_wo: jax.Array,
):
    return _impl(A_x, A_k_cache, A_v_cache, A_wq, A_wo, B_x, B_k_cache, B_v_cache, B_wq, B_wo)
```

```python
import functools
import jax
import jax.numpy as jnp
from jax import lax
from jax.experimental import pallas as pl
from jax.experimental.pallas import tpu as pltpu

B, D, HQ, HKV, SK, DH = 2, 448, 16, 8, 8192, 256
W = 2048
E = HQ * DH
NT = (((1,), (1,)), ((), ()))
NN = (((1,), (0,)), ((), ()))
WG = 4
WR = D // WG
WC = 512


def build(CH=256, NB=4, SR=8, compute=True, wo_chunks=(32, 32, 32, 16), QP=4, parts=2):
    CA = SK // CH
    CB = W // CH
    NA = B * CA
    NJ = NA + B * CB
    LA = NB - 1
    assert sum(wo_chunks) == WR
    wo_off = [sum(wo_chunks[:i]) for i in range(len(wo_chunks))]
    NWC = len(wo_chunks)
    NS = CH // SR

    def kernel(xa, xb, ak, av, awq, awo, bk, bv, bwq, bwo, o_hbm,
               kbuf, vbuf, wqbuf, wobuf, xbuf, q_scr, o_scr, m_scr, l_scr, acc_scr, outf_scr, out_scr,
               ksem, vsem, wqsem, wosem, xsem, osem):

        def decode(j, is_a):
            if is_a:
                return j // CA, j % CA, (j % CA) * CH
            jj = j - NA
            return jj // CB, jj % CB, (SK - W) + (jj % CB) * CH

        def issue(j, is_a, part, nparts):
            b, c, start = decode(j, is_a)
            slot = j % NB
            ks, vs = (ak, av) if is_a else (bk, bv)
            lo, hi = part * NS // nparts, (part + 1) * NS // nparts
            for i in range(lo, hi):
                s = i * SR
                st = start + s
                if not isinstance(st, int):
                    st = pl.multiple_of(st, SR)
                pltpu.make_async_copy(ks.at[b, :, pl.ds(st, SR), :], kbuf.at[slot, :, pl.ds(s, SR), :],
                                      ksem.at[slot]).start(priority=0)
                pltpu.make_async_copy(vs.at[b, :, pl.ds(st, SR), :], vbuf.at[slot, :, pl.ds(s, SR), :],
                                      vsem.at[slot]).start(priority=1)

        def w_descs(r0, nr):
            return [(r, c0) for r in range(r0, r0 + nr, 8) for c0 in range(0, E, WC)]

        def issue_w(ws, buf, sem_of, descs):
            for r, c0 in descs:
                for br in range(2):
                    pltpu.make_async_copy(ws[br].at[:, pl.ds(r, 8), pl.ds(c0, WC)],
                                          buf.at[br, :, pl.ds(r, 8), pl.ds(c0, WC)],
                                          sem_of(br)).start(priority=br)

        def issue_wo(c, part, nparts):
            d = w_descs(wo_off[c], wo_chunks[c])
            d = d[part * len(d) // nparts:(part + 1) * len(d) // nparts]
            issue_w((awo, bwo), wobuf, lambda br: wosem.at[br * NWC + c], d)

        def start_job(j, part, nparts):
            if isinstance(j, int):
                issue(j, j < NA, part, nparts)
            else:
                @pl.when(j < NA)
                def _():
                    issue(j, True, part, nparts)

                @pl.when(jnp.logical_and(j >= NA, j < NJ))
                def _():
                    issue(j, False, part, nparts)

                for t in range(min(LA, NWC)):
                    @pl.when(j == NJ + t)
                    def _():
                        issue_wo(t, part, nparts)

        xca = pltpu.make_async_copy(xa, xbuf.at[0], xsem.at[0])
        xcb = pltpu.make_async_copy(xb, xbuf.at[1], xsem.at[1])
        wqd = w_descs(0, WR)
        issue_w((awq, bwq), wqbuf, lambda br: wqsem.at[br], wqd[:8])
        xca.start()
        xcb.start()
        issue_w((awq, bwq), wqbuf, lambda br: wqsem.at[br], wqd[8:])

        q_scr[...] = jnp.zeros(q_scr.shape, q_scr.dtype)
        o_scr[...] = jnp.zeros(o_scr.shape, o_scr.dtype)

        start_job(0, 0, 1)

        def make_x(br):
            x2 = xbuf[br].astype(jnp.float32)
            rows = lax.broadcasted_iota(jnp.int32, (8, D), 0)
            x0 = jnp.broadcast_to(x2[0:1], (8, D))
            x1 = jnp.broadcast_to(x2[1:2], (8, D))
            return jnp.where(rows == 0, x0, jnp.where(rows == 1, x1, 0.0)).astype(jnp.bfloat16)

        def qproj(br, xx, piece):
            n = E // QP
            w = wqbuf[br, :, :, piece * n:(piece + 1) * n].reshape(D, n)
            q = lax.dot_general(xx, w, NN, preferred_element_type=jnp.float32)
            q = (q.astype(jnp.bfloat16).astype(jnp.float32) * (DH ** -0.5))
            for b in range(B):
                for hh in range(n // DH):
                    h = piece * (n // DH) + hh
                    q_scr[br, b, h // 2, h:h + 1, :] = q[b:b + 1, hh * DH:(hh + 1) * DH]

        xca.wait()
        xcb.wait()
        steps = [(br, pc) for br in range(2) for pc in range(QP)]
        PP = 4
        todo = [(jj, pt) for jj in range(1, LA) for pt in range(PP)]
        per = -(-len(todo) // len(steps)) if todo else 0
        xxs = {}
        for i, (br, pc) in enumerate(steps):
            if pc == 0:
                pltpu.make_async_copy(wqbuf.at[br], wqbuf.at[br], wqsem.at[br]).wait()
                xxs[br] = make_x(br)
            qproj(br, xxs[br], pc)
            for _ in range(per):
                if todo:
                    jj, pt = todo.pop(0)
                    start_job(jj, pt, PP)
        assert not todo

        def wait_k(slot):
            pltpu.make_async_copy(kbuf.at[slot], kbuf.at[slot], ksem.at[slot]).wait()

        def wait_v(slot):
            pltpu.make_async_copy(vbuf.at[slot], vbuf.at[slot], vsem.at[slot]).wait()

        def job(j, br, is_a):
            b, c, start = decode(j, is_a)
            slot = j % NB
            C = CA if is_a else CB

            @pl.when(c == 0)
            def _():
                m_scr[...] = jnp.full(m_scr.shape, -jnp.inf, jnp.float32)
                l_scr[...] = jnp.zeros(l_scr.shape, jnp.float32)
                acc_scr[...] = jnp.zeros(acc_scr.shape, jnp.float32)

            start_job(j + LA, 0, parts)
            wait_k(slot)
            if compute:
                s = None
                for g in range(HKV):
                    qg = q_scr[br, b, g].astype(jnp.bfloat16)
                    sg = lax.dot_general(qg, kbuf[slot, g], NT, preferred_element_type=jnp.float32)
                    s = sg if s is None else s + sg
                m_prev = m_scr[...]
                m_cur = jnp.max(s, axis=1, keepdims=True)
                m_new = jnp.maximum(m_prev, m_cur)
                alpha = jnp.exp(m_prev - m_new)
                p = jnp.exp(s - m_new[:, 0:1])
                l_scr[...] = alpha * l_scr[...] + jnp.sum(p, axis=1, keepdims=True)
                m_scr[...] = m_new
                pb = p.astype(jnp.bfloat16)
            if parts > 1:
                start_job(j + LA, 1, parts)
            wait_v(slot)
            if compute:
                grp = lax.broadcasted_iota(jnp.int32, (HQ, DH), 0) // 2
                acc = acc_scr[...] * alpha[:, 0:1]
                for g in range(HKV):
                    og = lax.dot_general(pb, vbuf[slot, g], NN, preferred_element_type=jnp.float32)
                    acc = acc + jnp.where(grp == g, og, 0.0)
                acc_scr[...] = acc

                @pl.when(c == C - 1)
                def _():
                    o = acc / l_scr[...][:, 0:1]
                    o = o.astype(jnp.bfloat16).astype(jnp.float32)
                    for h in range(HQ):
                        o_scr[br, pl.ds(b, 1), h * DH:(h + 1) * DH] = o[h:h + 1, :]

        def body_a(j, carry):
            job(j, 0, True)
            return carry
        lax.fori_loop(0, NA, body_a, 0)

        def body_b(j, carry):
            job(j, 1, False)
            return carry
        lax.fori_loop(NA, NJ, body_b, 0)

        pending = list(range(min(LA, NWC), NWC))
        obs = [o_scr[br].astype(jnp.bfloat16) for br in range(2)]
        for c in range(NWC):
            r0, nr = wo_off[c], wo_chunks[c]
            for br in range(2):
                if pending and c >= 0:
                    issue_wo(pending[0], br, 2)
                    if br == 1:
                        pending.pop(0)
                dst = wobuf.at[br, :, pl.ds(r0, nr), :]
                pltpu.make_async_copy(dst, dst, wosem.at[br * NWC + c]).wait()
                w = wobuf[br, :, r0:r0 + nr, :].reshape(WG * nr, E)
                part = lax.dot_general(obs[br], w, NT, preferred_element_type=jnp.float32)
                for g in range(WG):
                    f0 = br * D + g * WR + r0
                    outf_scr[:, f0:f0 + nr] = part[:, g * nr:(g + 1) * nr]
        out_scr[...] = outf_scr[0:B, :].astype(out_scr.dtype)
        oc = pltpu.make_async_copy(out_scr, o_hbm, osem.at[0])
        oc.start()
        oc.wait()

    @jax.jit
    def f(A_x, A_k_cache, A_v_cache, A_wq, A_wo, B_x, B_k_cache, B_v_cache, B_wq, B_wo):
        hbm = pl.BlockSpec(memory_space=pltpu.HBM)
        bf = jnp.bfloat16
        out = pl.pallas_call(
            kernel,
            out_shape=jax.ShapeDtypeStruct((B, 2 * D), bf),
            in_specs=[hbm] * 10,
            out_specs=hbm,
            scratch_shapes=[
                pltpu.VMEM((NB, HKV, CH, DH), bf),
                pltpu.VMEM((NB, HKV, CH, DH), bf),
                pltpu.VMEM((2, WG, WR, E), bf),
                pltpu.VMEM((2, WG, WR, E), bf),
                pltpu.VMEM((2, B, D), bf),
                pltpu.VMEM((2, B, HKV, HQ, DH), jnp.float32),
                pltpu.VMEM((2, 8, E), jnp.float32),
                pltpu.VMEM((HQ, 128), jnp.float32),
                pltpu.VMEM((HQ, 128), jnp.float32),
                pltpu.VMEM((HQ, DH), jnp.float32),
                pltpu.VMEM((8, 2 * D), jnp.float32),
                pltpu.VMEM((B, 2 * D), bf),
                pltpu.SemaphoreType.DMA((NB,)),
                pltpu.SemaphoreType.DMA((NB,)),
                pltpu.SemaphoreType.DMA((2,)),
                pltpu.SemaphoreType.DMA((2 * NWC,)),
                pltpu.SemaphoreType.DMA((2,)),
                pltpu.SemaphoreType.DMA((1,)),
            ],
            compiler_params=pltpu.CompilerParams(vmem_limit_bytes=100 * 1024 * 1024),
        )(A_x.reshape(B, D), B_x.reshape(B, D), A_k_cache, A_v_cache,
          A_wq.reshape(WG, WR, E), A_wo.T.reshape(WG, WR, E),
          B_k_cache, B_v_cache,
          B_wq.reshape(WG, WR, E), B_wo.T.reshape(WG, WR, E))
        return out.reshape(B, 1, 2 * D)
    return f


_impl = build(wo_chunks=(32, 32, 16, 16, 16))


@jax.jit
def pallas_concat_heads__gqa_block_cached__sliding_block_cached__decode_kernel(
    A_x: jax.Array,
    A_k_cache: jax.Array,
    A_v_cache: jax.Array,
    A_wq: jax.Array,
    A_wo: jax.Array,
    B_x: jax.Array,
    B_k_cache: jax.Array,
    B_v_cache: jax.Array,
    B_wq: jax.Array,
    B_wo: jax.Array,
):
    return _impl(A_x, A_k_cache, A_v_cache, A_wq, A_wo, B_x, B_k_cache, B_v_cache, B_wq, B_wo)
```

```python
import functools
import jax
import jax.numpy as jnp
from jax import lax
from jax.experimental import pallas as pl
from jax.experimental.pallas import tpu as pltpu

B, D, HQ, HKV, SK, DH = 2, 448, 16, 8, 8192, 256
W = 2048
E = HQ * DH
NT = (((1,), (1,)), ((), ()))
NN = (((1,), (0,)), ((), ()))
WG = 4
WR = D // WG
WC = 512
G = HKV

DEF_GROUPS = (
    ((0, 1), 0, 32, 0, 4096),
    ((0, 1), 32, 32, 0, 4096),
    ((0,), 64, 32, 0, 4096),
    ((1,), 64, 16, 0, 4096),
    ((0,), 96, 16, 0, 4096),
    ((1,), 80, 16, 0, 4096),
    ((1,), 96, 16, 0, 2560),
    ((1,), 96, 16, 2560, 1024),
    ((1,), 96, 16, 3584, 512),
)


def build(CH=256, L=3, SR=8, compute=True, QP=4, parts=2, groups=DEF_GROUPS, qb='mid',
          stage_rows=(32, 32, 16, 16, 16), post=(0, 1), WCQ=128, WCO=(512, 512, 512, 512, 512), wq_mode='pair'):
    WC = 128
    NB = L + 1
    CA = SK // CH
    CB = W // CH
    NA = B * CA
    NJ = NA + B * CB
    NS = CH // SR
    NGR = len(groups)
    assert sum(stage_rows) == WR
    st_off = [sum(stage_rows[:i]) for i in range(len(stage_rows))]
    NST = len(stage_rows)
    gmap = {}
    for gi, (brs, r0, nr, c0, cw) in enumerate(groups):
        assert r0 % 16 == 0 and nr % 16 == 0 and c0 % WC == 0 and cw % WC == 0
        for br in brs:
            for r in range(r0, r0 + nr, 8):
                for c in range(c0, c0 + cw, WC):
                    assert (br, r, c) not in gmap
                    gmap[(br, r, c)] = gi
    assert len(gmap) == 2 * (WR // 8) * (E // WC)
    nrot = 0
    while nrot < min(L, NST) and groups[nrot] == ((0, 1), st_off[nrot], stage_rows[nrot], 0, E):
        nrot += 1
    NSEM = L + NGR - nrot
    for t in range(NST):
        for br in range(2):
            for r in range(st_off[t], st_off[t] + stage_rows[t], 8):
                for c0 in range(0, E, WCO[t]):
                    assert len({gmap[(br, r, c)] for c in range(c0, c0 + WCO[t], WC)}) == 1
    assert len(post) == max(NST - L, 0)

    def kernel(xa, xb, ak, av, awq, awo, bk, bv, bwq, bwo, o_hbm,
               kvbuf, wqbuf, wobuf, xbuf, q_scr, o_scr, m_scr, l_scr, acc_scr, outf_scr, out_scr, pp_scr,
               sem):
        def decode(j, is_a):
            if is_a:
                return j // CA, j % CA, (j % CA) * CH
            jj = j - NA
            return jj // CB, jj % CB, (SK - W) + (jj % CB) * CH

        def issue(j, is_a, part, nparts):
            b, c, start = decode(j, is_a)
            slot = j % NB
            sm = sem.at[(j + 1) % L]
            ks, vs = (ak, av) if is_a else (bk, bv)
            lo, hi = part * NS // nparts, (part + 1) * NS // nparts
            for i in range(lo, hi):
                s = i * SR
                st = start + s
                if not isinstance(st, int):
                    st = pl.multiple_of(st, SR)
                pltpu.make_async_copy(ks.at[b, :, pl.ds(st, SR), :], kvbuf.at[slot, 0, :, pl.ds(s, SR), :],
                                      sm).start(priority=0)
                pltpu.make_async_copy(vs.at[b, :, pl.ds(st, SR), :], kvbuf.at[slot, 1, :, pl.ds(s, SR), :],
                                      sm).start(priority=1)

        def issue_w(ws, buf, descs, sem_of, wc=WC):
            for r, c0 in descs:
                for br in range(2):
                    pltpu.make_async_copy(ws[br].at[:, pl.ds(r, 8), pl.ds(c0, wc)],
                                          buf.at[br, :, pl.ds(r, 8), pl.ds(c0, wc)],
                                          sem_of(br, r, c0)).start(priority=br)

        def issue_wq_grp(descs):
            for br, r, c0 in descs:
                for t in range(2):
                    pltpu.make_async_copy((awq, bwq)[br].at[pl.ds(2 * t, 2), pl.ds(r, 8), pl.ds(c0, WCQ)],
                                          wqbuf.at[br, pl.ds(2 * t, 2), pl.ds(r, 8), pl.ds(c0, WCQ)],
                                          s0).start(priority=t)

        def group_sem(gi):
            if gi < nrot:
                return sem.at[(1 + NJ + gi) % L]
            return sem.at[L + gi - nrot]

        def stage_descs(t):
            r0, nr = st_off[t], stage_rows[t]
            wc = WCO[t]
            if t < NST - 1:
                return [(r, cc) for r in range(r0, r0 + nr, 8) for cc in range(0, E, wc)]
            return [(r, cc) for cc in range(0, E, wc) for r in range(r0, r0 + nr, 8)]

        def issue_wo(t, part, nparts):
            d = stage_descs(t)
            issue_w((awo, bwo), wobuf, d[part * len(d) // nparts:(part + 1) * len(d) // nparts],
                    lambda br, r, c: group_sem(gmap[(br, r, c)]), WCO[t])

        def start_job(j, part, nparts):
            if isinstance(j, int):
                issue(j, j < NA, part, nparts)
            else:
                @pl.when(j < NA)
                def _():
                    issue(j, True, part, nparts)

                @pl.when(jnp.logical_and(j >= NA, j < NJ))
                def _():
                    issue(j, False, part, nparts)

                for t in range(min(L, NST)):
                    @pl.when(j == NJ + t)
                    def _():
                        issue_wo(t, part, nparts)

        s0 = sem.at[0]
        xca = pltpu.make_async_copy(xa, xbuf.at[0], s0)
        xcb = pltpu.make_async_copy(xb, xbuf.at[1], s0)
        if wq_mode == 'pair':
            wqd = [(r, c0) for r in range(0, WR, 8) for c0 in range(0, E, WCQ)]
            issue_w((awq, bwq), wqbuf, wqd[:8], lambda *_: s0, WCQ)
            xca.start()
            xcb.start()
            issue_w((awq, bwq), wqbuf, wqd[8:], lambda *_: s0, WCQ)
        else:
            wqd = [(br, r, c0) for br in range(2) for r in range(0, WR, 8) for c0 in range(0, E, WCQ)]
            issue_wq_grp(wqd[:8])
            xca.start()
            xcb.start()
            issue_wq_grp(wqd[8:])

        o_scr[...] = jnp.zeros(o_scr.shape, o_scr.dtype)

        for jj in range(L - 1):
            start_job(jj, 0, 1)

        def make_x(br):
            x2 = xbuf[br].astype(jnp.float32)
            rows = lax.broadcasted_iota(jnp.int32, (8, D), 0)
            x0 = jnp.broadcast_to(x2[0:1], (8, D))
            x1 = jnp.broadcast_to(x2[1:2], (8, D))
            return jnp.where(rows == 0, x0, jnp.where(rows == 1, x1, 0.0)).astype(jnp.bfloat16)

        def qproj(br, xx, piece):
            n = E // QP
            w = wqbuf[br, :, :, piece * n:(piece + 1) * n].reshape(D, n)
            q = lax.dot_general(xx, w, NN, preferred_element_type=jnp.float32)
            q = (q.astype(jnp.bfloat16).astype(jnp.float32) * (DH ** -0.5))
            for b in range(B):
                for hh in range(n // DH):
                    h = piece * (n // DH) + hh
                    q_scr[br, b, h:h + 1, :] = q[b:b + 1, hh * DH:(hh + 1) * DH]

        xca.wait()
        xcb.wait()
        pltpu.make_async_copy(wqbuf, wqbuf, s0).wait()
        xx = make_x(0)
        for pc in range(QP):
            start_job(L - 1, pc, QP)
            qproj(0, xx, pc)
        if qb == 'early':
            xx = make_x(1)
            for pc in range(QP):
                qproj(1, xx, pc)

        def job(j, br, is_a):
            b, c, start = decode(j, is_a)
            slot = j % NB
            C = CA if is_a else CB

            @pl.when(c == 0)
            def _():
                m_scr[...] = jnp.full(m_scr.shape, -jnp.inf, jnp.float32)
                l_scr[...] = jnp.zeros(l_scr.shape, jnp.float32)
                acc_scr[...] = jnp.zeros(acc_scr.shape, jnp.float32)

            grp = lax.broadcasted_iota(jnp.int32, (HQ, DH), 0) // 2
            q16 = q_scr[br, b]
            pltpu.make_async_copy(kvbuf.at[slot], kvbuf.at[slot], sem.at[(j + 1) % L]).wait()
            start_job(j + L, 0, parts)
            if compute:
                s = None
                for g in range(G):
                    qg = jnp.where(grp == g, q16, 0.0).astype(jnp.bfloat16)
                    sg = lax.dot_general(qg, kvbuf[slot, 0, g], NT, preferred_element_type=jnp.float32)
                    s = sg if s is None else s + sg
                m_prev = m_scr[...]
                m_cur = jnp.max(s, axis=1, keepdims=True)
                m_new = jnp.maximum(m_prev, m_cur)
                alpha = jnp.exp(m_prev - m_new)
                p = jnp.exp(s - m_new[:, 0:1])
                l_new = alpha * l_scr[...] + jnp.sum(p, axis=1, keepdims=True)
                l_scr[...] = l_new
                m_scr[...] = m_new
                pb = p.astype(jnp.bfloat16)
            if parts > 1:
                start_job(j + L, 1, parts)
            if compute:
                acc = acc_scr[...] * alpha[:, 0:1]
                for g in range(G):
                    og = lax.dot_general(pb, kvbuf[slot, 1, g], NN, preferred_element_type=jnp.float32)
                    acc = acc + jnp.where(grp == g, og, 0.0)
                acc_scr[...] = acc

                @pl.when(c == C - 1)
                def _():
                    o = acc / l_new[:, 0:1]
                    o = o.astype(jnp.bfloat16).astype(jnp.float32)
                    for h in range(HQ):
                        o_scr[br, pl.ds(b, 1), h * DH:(h + 1) * DH] = o[h:h + 1, :]

        def body_a(j, carry):
            job(j, 0, True)
            return carry
        lax.fori_loop(0, NA, body_a, 0)

        if qb == 'mid':
            xx = make_x(1)
            for pc in range(QP):
                qproj(1, xx, pc)

        def body_b(j, carry):
            job(j, 1, False)
            return carry
        lax.fori_loop(NA, NJ, body_b, 0)

        obs = [o_scr[br].astype(jnp.bfloat16) for br in range(2)]

        def scatter(br, part, r0, nr):
            for g in range(WG):
                f0 = br * D + g * WR + r0
                outf_scr[:, f0:f0 + nr] = part[:, g * nr:(g + 1) * nr]

        for gi, (brs, r0, nr, c0, cw) in enumerate(groups):
            for i, pg in enumerate(post):
                if pg == gi:
                    issue_wo(L + i, 0, 1)
            dst = wobuf.at[pl.ds(brs[0], len(brs)), :, pl.ds(r0, nr), pl.ds(c0, cw)]
            pltpu.make_async_copy(dst, dst, group_sem(gi)).wait()
            for br in brs:
                w = wobuf[br, :, r0:r0 + nr, c0:c0 + cw].reshape(WG * nr, cw)
                pt = lax.dot_general(obs[br][:, c0:c0 + cw], w, NT, preferred_element_type=jnp.float32)
                if c0 > 0:
                    pt = pt + pp_scr[br, :, 0:WG * nr]
                if c0 + cw < E:
                    pp_scr[br, :, 0:WG * nr] = pt
                else:
                    scatter(br, pt, r0, nr)
        out_scr[...] = outf_scr[0:B, :].astype(out_scr.dtype)
        oc = pltpu.make_async_copy(out_scr, o_hbm, s0)
        oc.start()
        oc.wait()

    @jax.jit
    def f(A_x, A_k_cache, A_v_cache, A_wq, A_wo, B_x, B_k_cache, B_v_cache, B_wq, B_wo):
        hbm = pl.BlockSpec(memory_space=pltpu.HBM)
        bf = jnp.bfloat16
        out = pl.pallas_call(
            kernel,
            out_shape=jax.ShapeDtypeStruct((B, 2 * D), bf),
            in_specs=[hbm] * 10,
            out_specs=hbm,
            scratch_shapes=[
                pltpu.VMEM((NB, 2, G, CH, DH), bf),
                pltpu.VMEM((2, WG, WR, E), bf),
                pltpu.VMEM((2, WG, WR, E), bf),
                pltpu.VMEM((2, B, D), bf),
                pltpu.VMEM((2, B, HQ, DH), jnp.float32),
                pltpu.VMEM((2, 8, E), jnp.float32),
                pltpu.VMEM((HQ, 128), jnp.float32),
                pltpu.VMEM((HQ, 128), jnp.float32),
                pltpu.VMEM((HQ, DH), jnp.float32),
                pltpu.VMEM((8, 2 * D), jnp.float32),
                pltpu.VMEM((B, 2 * D), bf),
                pltpu.VMEM((2, 8, 256), jnp.float32),
                pltpu.SemaphoreType.DMA((NSEM,)),
            ],
            compiler_params=pltpu.CompilerParams(vmem_limit_bytes=100 * 1024 * 1024),
        )(A_x.reshape(B, D), B_x.reshape(B, D), A_k_cache, A_v_cache,
          A_wq.reshape(WG, WR, E), A_wo.T.reshape(WG, WR, E),
          B_k_cache, B_v_cache,
          B_wq.reshape(WG, WR, E), B_wo.T.reshape(WG, WR, E))
        return out.reshape(B, 1, 2 * D)
    return f


_impl = build()


@jax.jit
def pallas_concat_heads__gqa_block_cached__sliding_block_cached__decode_kernel(
    A_x: jax.Array,
    A_k_cache: jax.Array,
    A_v_cache: jax.Array,
    A_wq: jax.Array,
    A_wo: jax.Array,
    B_x: jax.Array,
    B_k_cache: jax.Array,
    B_v_cache: jax.Array,
    B_wq: jax.Array,
    B_wo: jax.Array,
):
    return _impl(A_x, A_k_cache, A_v_cache, A_wq, A_wo, B_x, B_k_cache, B_v_cache, B_wq, B_wo)
```

```python
import jax
import jax.numpy as jnp
from jax import lax
from jax.experimental import pallas as pl
from jax.experimental.pallas import tpu as pltpu

B, D, HQ, HKV, SK, DH = 2, 448, 16, 8, 8192, 256
WIN = min(4096, max(256, SK // 4))
E = HQ * DH
REP = HQ // HKV
NT = (((1,), (1,)), ((), ()))
NN = (((1,), (0,)), ((), ()))

CH = 256
SR = 8
NS = CH // SR
L = 3
NB = L + 1
CA = SK // CH
CB = WIN // CH
NA = B * CA
NJ = NA + B * CB

WG = 4
WR = D // WG
WCQ = 128
WCO = 512
QP = 4

STAGE_ROWS = (32, 32, 16, 16, 16)
STAGE_OFF = tuple(sum(STAGE_ROWS[:i]) for i in range(len(STAGE_ROWS)))


def _rot(t):
    return (1 + NJ + t) % L


WO_GROUPS = (
    ((0, 1), 0, 32, 0, E, _rot(0), 3),
    ((0, 1), 32, 32, 0, E, _rot(1), None),
    ((0,), 64, 32, 0, E, L, None),
    ((1,), 64, 16, 0, E, _rot(2), None),
    ((0,), 96, 16, 0, E, L + 1, None),
    ((1,), 80, 16, 0, E, _rot(0), None),
    ((1,), 96, 16, 0, 2560, L + 2, None),
    ((1,), 96, 16, 2560, 1024, L + 3, None),
    ((1,), 96, 16, 3584, 512, L + 4, None),
)
NSEM = L + 5
_WO_SEM = {}
for _brs, _r0, _nr, _c0, _cw, _si, _ in WO_GROUPS:
    for _br in _brs:
        for _r in range(_r0, _r0 + _nr, 8):
            for _c in range(_c0, _c0 + _cw, WCO):
                assert (_br, _r, _c) not in _WO_SEM
                _WO_SEM[(_br, _r, _c)] = _si
assert len(_WO_SEM) == 2 * (WR // 8) * (E // WCO)


def _kernel(xa, xb, ak, av, awq, awo, bk, bv, bwq, bwo, o_ref,
            kvbuf, wqbuf, wobuf, xbuf, q_scr, o_scr, m_scr, l_scr, acc_scr, outf_scr, pp_scr,
            sem):
    f32, bf16 = jnp.float32, jnp.bfloat16

    def decode(j, is_a):
        if is_a:
            return j // CA, j % CA, (j % CA) * CH
        jj = j - NA
        return jj // CB, jj % CB, (SK - WIN) + (jj % CB) * CH

    def issue_kv(j, is_a, part, nparts):
        b, _, start = decode(j, is_a)
        slot = j % NB
        sm = sem.at[(j + 1) % L]
        ks, vs = (ak, av) if is_a else (bk, bv)
        for i in range(part * NS // nparts, (part + 1) * NS // nparts):
            s = i * SR
            st = start + s
            if not isinstance(st, int):
                st = pl.multiple_of(st, SR)
            pltpu.make_async_copy(ks.at[b, :, pl.ds(st, SR), :], kvbuf.at[slot, 0, :, pl.ds(s, SR), :],
                                  sm).start(priority=0)
            pltpu.make_async_copy(vs.at[b, :, pl.ds(st, SR), :], kvbuf.at[slot, 1, :, pl.ds(s, SR), :],
                                  sm).start(priority=1)

    def issue_w(ws, buf, descs, sem_of, wc):
        for r, c0 in descs:
            for br in range(2):
                pltpu.make_async_copy(ws[br].at[:, pl.ds(r, 8), pl.ds(c0, wc)],
                                      buf.at[br, :, pl.ds(r, 8), pl.ds(c0, wc)],
                                      sem_of(br, r, c0)).start(priority=br)

    def issue_wo(t, part=0, nparts=1):
        rows = range(STAGE_OFF[t], STAGE_OFF[t] + STAGE_ROWS[t], 8)
        cols = range(0, E, WCO)
        if t < len(STAGE_ROWS) - 1:
            d = [(r, c) for r in rows for c in cols]
        else:
            d = [(r, c) for c in cols for r in rows]
        issue_w((awo, bwo), wobuf, d[part * len(d) // nparts:(part + 1) * len(d) // nparts],
                lambda br, r, c: sem.at[_WO_SEM[(br, r, c)]], WCO)

    def start_job(j, part, nparts):
        if isinstance(j, int):
            issue_kv(j, j < NA, part, nparts)
            return

        @pl.when(j < NA)
        def _():
            issue_kv(j, True, part, nparts)

        @pl.when(jnp.logical_and(j >= NA, j < NJ))
        def _():
            issue_kv(j, False, part, nparts)

        for t in range(L):
            @pl.when(j == NJ + t)
            def _():
                issue_wo(t, part, nparts)

    s0 = sem.at[0]
    xca = pltpu.make_async_copy(xa, xbuf.at[0], s0)
    xcb = pltpu.make_async_copy(xb, xbuf.at[1], s0)
    wqd = [(r, c0) for r in range(0, WR, 8) for c0 in range(0, E, WCQ)]
    issue_w((awq, bwq), wqbuf, wqd[:8], lambda *_: s0, WCQ)
    xca.start()
    xcb.start()
    issue_w((awq, bwq), wqbuf, wqd[8:], lambda *_: s0, WCQ)

    o_scr[...] = jnp.zeros(o_scr.shape, o_scr.dtype)

    for jj in range(L - 1):
        start_job(jj, 0, 1)

    def make_x(br):
        x2 = xbuf[br].astype(f32)
        rows = lax.broadcasted_iota(jnp.int32, (8, D), 0)
        x0 = jnp.broadcast_to(x2[0:1], (8, D))
        x1 = jnp.broadcast_to(x2[1:2], (8, D))
        return jnp.where(rows == 0, x0, jnp.where(rows == 1, x1, 0.0)).astype(bf16)

    def qproj(br, xx, piece):
        n = E // QP
        w = wqbuf[br, :, :, piece * n:(piece + 1) * n].reshape(D, n)
        q = lax.dot_general(xx, w, NN, preferred_element_type=f32)
        q = q.astype(bf16).astype(f32) * (DH ** -0.5)
        for b in range(B):
            for hh in range(n // DH):
                h = piece * (n // DH) + hh
                q_scr[br, b, h:h + 1, :] = q[b:b + 1, hh * DH:(hh + 1) * DH]

    xca.wait()
    xcb.wait()
    pltpu.make_async_copy(wqbuf, wqbuf, s0).wait()
    xx = make_x(0)
    for pc in range(QP):
        start_job(L - 1, pc, QP)
        qproj(0, xx, pc)

    def job(j, br, is_a):
        b, c, _ = decode(j, is_a)
        slot = j % NB
        last = (CA if is_a else CB) - 1

        @pl.when(c == 0)
        def _():
            m_scr[...] = jnp.full(m_scr.shape, -jnp.inf, f32)
            l_scr[...] = jnp.zeros(l_scr.shape, f32)
            acc_scr[...] = jnp.zeros(acc_scr.shape, f32)

        grp = lax.broadcasted_iota(jnp.int32, (HQ, DH), 0) // REP
        q16 = q_scr[br, b]
        pltpu.make_async_copy(kvbuf.at[slot], kvbuf.at[slot], sem.at[(j + 1) % L]).wait()
        start_job(j + L, 0, 2)

        s = None
        for g in range(HKV):
            qg = jnp.where(grp == g, q16, 0.0).astype(bf16)
            sg = lax.dot_general(qg, kvbuf[slot, 0, g], NT, preferred_element_type=f32)
            s = sg if s is None else s + sg
        m_prev = m_scr[...]
        m_new = jnp.maximum(m_prev, jnp.max(s, axis=1, keepdims=True))
        alpha = jnp.exp(m_prev - m_new)
        p = jnp.exp(s - m_new[:, 0:1])
        l_new = alpha * l_scr[...] + jnp.sum(p, axis=1, keepdims=True)
        l_scr[...] = l_new
        m_scr[...] = m_new
        pb = p.astype(bf16)

        start_job(j + L, 1, 2)

        acc = acc_scr[...] * alpha[:, 0:1]
        for g in range(HKV):
            og = lax.dot_general(pb, kvbuf[slot, 1, g], NN, preferred_element_type=f32)
            acc = acc + jnp.where(grp == g, og, 0.0)
        acc_scr[...] = acc

        @pl.when(c == last)
        def _():
            o = (acc / l_new[:, 0:1]).astype(bf16).astype(f32)
            for h in range(HQ):
                o_scr[br, pl.ds(b, 1), h * DH:(h + 1) * DH] = o[h:h + 1, :]

    def body_a(j, carry):
        job(j, 0, True)
        return carry

    def body_b(j, carry):
        job(j, 1, False)
        return carry

    lax.fori_loop(0, NA, body_a, 0)

    xx = make_x(1)
    for pc in range(QP):
        qproj(1, xx, pc)

    lax.fori_loop(NA, NJ, body_b, 0)

    obs = [o_scr[br].astype(bf16) for br in range(2)]
    for gi, (brs, r0, nr, c0, cw, si, then_issue) in enumerate(WO_GROUPS):
        if gi == 1:
            issue_wo(4)
        dst = wobuf.at[pl.ds(brs[0], len(brs)), :, pl.ds(r0, nr), pl.ds(c0, cw)]
        pltpu.make_async_copy(dst, dst, sem.at[si]).wait()
        if then_issue is not None:
            issue_wo(then_issue)
        for br in brs:
            w = wobuf[br, :, r0:r0 + nr, c0:c0 + cw].reshape(WG * nr, cw)
            pt = lax.dot_general(obs[br][:, c0:c0 + cw], w, NT, preferred_element_type=f32)
            if c0 > 0:
                pt = pt + pp_scr[:, 0:WG * nr]
            if c0 + cw < E:
                pp_scr[:, 0:WG * nr] = pt
            else:
                for g in range(WG):
                    f0 = br * D + g * WR + r0
                    outf_scr[:, f0:f0 + nr] = pt[:, g * nr:(g + 1) * nr]

    o_ref[...] = outf_scr[0:B, :].astype(o_ref.dtype)


@jax.jit
def pallas_concat_heads__gqa_block_cached__sliding_block_cached__decode_kernel(
    A_x: jax.Array,
    A_k_cache: jax.Array,
    A_v_cache: jax.Array,
    A_wq: jax.Array,
    A_wo: jax.Array,
    B_x: jax.Array,
    B_k_cache: jax.Array,
    B_v_cache: jax.Array,
    B_wq: jax.Array,
    B_wo: jax.Array,
):
    hbm = pl.BlockSpec(memory_space=pltpu.HBM)
    bf16, f32 = jnp.bfloat16, jnp.float32
    out = pl.pallas_call(
        _kernel,
        out_shape=jax.ShapeDtypeStruct((B, 2 * D), bf16),
        in_specs=[hbm] * 10,
        out_specs=pl.BlockSpec(memory_space=pltpu.VMEM),
        scratch_shapes=[
            pltpu.VMEM((NB, 2, HKV, CH, DH), bf16),
            pltpu.VMEM((2, WG, WR, E), bf16),
            pltpu.VMEM((2, WG, WR, E), bf16),
            pltpu.VMEM((2, B, D), bf16),
            pltpu.VMEM((2, B, HQ, DH), f32),
            pltpu.VMEM((2, 8, E), f32),
            pltpu.VMEM((HQ, 128), f32),
            pltpu.VMEM((HQ, 128), f32),
            pltpu.VMEM((HQ, DH), f32),
            pltpu.VMEM((8, 2 * D), f32),
            pltpu.VMEM((8, 128), f32),
            pltpu.SemaphoreType.DMA((NSEM,)),
        ],
        compiler_params=pltpu.CompilerParams(vmem_limit_bytes=64 * 1024 * 1024),
    )(A_x.reshape(B, D), B_x.reshape(B, D), A_k_cache, A_v_cache,
      A_wq.reshape(WG, WR, E), A_wo.T.reshape(WG, WR, E),
      B_k_cache, B_v_cache,
      B_wq.reshape(WG, WR, E), B_wo.T.reshape(WG, WR, E))
    return out.reshape(B, 1, 2 * D)
```

```python
import jax
import jax.numpy as jnp
from jax import lax
from jax.experimental import pallas as pl
from jax.experimental.pallas import tpu as pltpu

B, D, HQ, HKV, SK, DH = 2, 448, 16, 8, 8192, 256
WIN = min(4096, max(256, SK // 4))
E = HQ * DH
REP = HQ // HKV
NT = (((1,), (1,)), ((), ()))
NN = (((1,), (0,)), ((), ()))

CH = 256
SR = 8
NS = CH // SR
L = 3
NB = L + 1
G = 8
BLK = 2048
NBLK = SK // BLK
CS = BLK // CH
NBA = B * HKV * NBLK
NBB = B * HKV
NSA = NBA // G
NSB = NBB // G
NA = NSA * CS
NJ = NA + NSB * CS
SHIFT_A = 2
SHIFT_B = 0
assert WIN == BLK


def _places(br, hk):
    if br == 0:
        ks = [(hk * NBLK + k - SHIFT_A) % NBA for k in range(NBLK)]
        return [(k // G, k % G) for k in ks]
    k = (hk - SHIFT_B) % NBB
    return [(NSA + k // G, k % G)]


WG = 4
WR = D // WG
WCQ = 128
WCO = 512
QP = 4

STAGE_ROWS = (32, 32, 16, 16, 16)
STAGE_OFF = tuple(sum(STAGE_ROWS[:i]) for i in range(len(STAGE_ROWS)))


def _rot(t):
    return (1 + NJ + t) % L


WO_GROUPS = (
    ((0, 1), 0, 32, 0, E, _rot(0), 3),
    ((0, 1), 32, 32, 0, E, _rot(1), None),
    ((0,), 64, 32, 0, E, L, None),
    ((1,), 64, 16, 0, E, _rot(2), None),
    ((0,), 96, 16, 0, E, L + 1, None),
    ((1,), 80, 16, 0, E, _rot(0), None),
    ((1,), 96, 16, 0, 2560, L + 2, None),
    ((1,), 96, 16, 2560, 1024, L + 3, None),
    ((1,), 96, 16, 3584, 512, L + 4, None),
)
NSEM = L + 5
_WO_SEM = {}
for _brs, _r0, _nr, _c0, _cw, _si, _ in WO_GROUPS:
    for _br in _brs:
        for _r in range(_r0, _r0 + _nr, 8):
            for _c in range(_c0, _c0 + _cw, WCO):
                assert (_br, _r, _c) not in _WO_SEM
                _WO_SEM[(_br, _r, _c)] = _si
assert len(_WO_SEM) == 2 * (WR // 8) * (E // WCO)


def _kernel(xa, xb, ak, av, awq, awo, bk, bv, bwq, bwo, o_ref,
            kvbuf, wqbuf, wobuf, xbuf, q_scr, o_scr, m_scr, l_scr, acc_scr,
            pm_scr, pl_scr, pa_scr, outf_scr, pp_scr, sem):
    f32, bf16 = jnp.float32, jnp.bfloat16

    def issue_kv(j, is_a, wrap, part, nparts):
        n, shift = (NBA, SHIFT_A) if is_a else (NBB, SHIFT_B)
        w = j // CS - (0 if is_a else NSA)
        start = (j % CS) * CH + (0 if is_a else SK - WIN)
        slot = j % NB
        sm = sem.at[(j + 1) % L]
        if wrap:
            pieces = [(n - (G - shift), 0, G - shift), (0, G - shift, shift)]
        else:
            pieces = [(shift + G * w, 0, G)]
        for i in range(part * NS // nparts, (part + 1) * NS // nparts):
            s = i * SR
            st = start + s
            if not isinstance(st, int):
                st = pl.multiple_of(st, SR)
            for kv, src in enumerate((ak, av) if is_a else (bk, bv)):
                for g0, d0, ng in pieces:
                    pltpu.make_async_copy(src.at[pl.ds(g0, ng), pl.ds(st, SR), :],
                                          kvbuf.at[slot, kv, pl.ds(d0, ng), pl.ds(s, SR), :],
                                          sm).start(priority=kv)

    def issue_w(ws, buf, descs, sem_of, wc):
        for r, c0 in descs:
            for br in range(2):
                pltpu.make_async_copy(ws[br].at[:, pl.ds(r, 8), pl.ds(c0, wc)],
                                      buf.at[br, :, pl.ds(r, 8), pl.ds(c0, wc)],
                                      sem_of(br, r, c0)).start(priority=br)

    def issue_wo(t, part=0, nparts=1):
        rows = range(STAGE_OFF[t], STAGE_OFF[t] + STAGE_ROWS[t], 8)
        cols = range(0, E, WCO)
        if t < len(STAGE_ROWS) - 1:
            d = [(r, c) for r in rows for c in cols]
        else:
            d = [(r, c) for c in cols for r in rows]
        issue_w((awo, bwo), wobuf, d[part * len(d) // nparts:(part + 1) * len(d) // nparts],
                lambda br, r, c: sem.at[_WO_SEM[(br, r, c)]], WCO)

    ranges = []
    for is_a, j0, nseq, shift in ((True, 0, NSA, SHIFT_A), (False, NA, NSB, SHIFT_B)):
        jw = j0 + (nseq - 1) * CS if shift else j0 + nseq * CS
        ranges.append((j0, jw, is_a, False))
        if shift:
            ranges.append((jw, j0 + nseq * CS, is_a, True))

    def start_job(j, part, nparts):
        if isinstance(j, int):
            for lo, hi, is_a, wrap in ranges:
                if lo <= j < hi:
                    issue_kv(j, is_a, wrap, part, nparts)
            return

        for lo, hi, is_a, wrap in ranges:
            @pl.when(jnp.logical_and(j >= lo, j < hi))
            def _():
                issue_kv(j, is_a, wrap, part, nparts)

        for t in range(L):
            @pl.when(j == NJ + t)
            def _():
                issue_wo(t, part, nparts)

    s0 = sem.at[0]
    xca = pltpu.make_async_copy(xa, xbuf.at[0], s0)
    xcb = pltpu.make_async_copy(xb, xbuf.at[1], s0)
    wqd = [(r, c0) for r in range(0, WR, 8) for c0 in range(0, E, WCQ)]
    issue_w((awq, bwq), wqbuf, wqd[:8], lambda *_: s0, WCQ)
    xca.start()
    xcb.start()
    issue_w((awq, bwq), wqbuf, wqd[8:], lambda *_: s0, WCQ)

    o_scr[...] = jnp.zeros(o_scr.shape, o_scr.dtype)

    for jj in range(L - 1):
        start_job(jj, 0, 1)

    def make_x(br):
        x2 = xbuf[br].astype(f32)
        rows = lax.broadcasted_iota(jnp.int32, (8, D), 0)
        x0 = jnp.broadcast_to(x2[0:1], (8, D))
        x1 = jnp.broadcast_to(x2[1:2], (8, D))
        return jnp.where(rows == 0, x0, jnp.where(rows == 1, x1, 0.0)).astype(bf16)

    def qproj(br, xx, piece):
        n = E // QP
        w = wqbuf[br, :, :, piece * n:(piece + 1) * n].reshape(D, n)
        q = lax.dot_general(xx, w, NN, preferred_element_type=f32)
        q = q.astype(bf16).astype(f32) * (DH ** -0.5)
        for b in range(B):
            for hh in range(n // DH):
                h = piece * (n // DH) + hh
                qh = q[b:b + 1, hh * DH:(hh + 1) * DH]
                for w, i in _places(br, b * HKV + h // REP):
                    row = REP * i + h % REP
                    q_scr[w, row:row + 1, :] = qh

    xca.wait()
    xcb.wait()
    pltpu.make_async_copy(wqbuf, wqbuf, s0).wait()
    xx = make_x(0)
    for pc in range(QP):
        start_job(L - 1, pc, QP)
        qproj(0, xx, pc)

    def job(j, carry):
        w = j // CS
        c = j % CS
        slot = j % NB

        @pl.when(c == 0)
        def _():
            m_scr[...] = jnp.full(m_scr.shape, -jnp.inf, f32)
            l_scr[...] = jnp.zeros(l_scr.shape, f32)
            acc_scr[...] = jnp.zeros(acc_scr.shape, f32)

        grp = lax.broadcasted_iota(jnp.int32, (HQ, DH), 0) // REP
        q16 = q_scr[w]
        pltpu.make_async_copy(kvbuf.at[slot], kvbuf.at[slot], sem.at[(j + 1) % L]).wait()
        start_job(j + L, 0, 2)

        s = None
        for g in range(G):
            qg = jnp.where(grp == g, q16, 0.0).astype(bf16)
            sg = lax.dot_general(qg, kvbuf[slot, 0, g], NT, preferred_element_type=f32)
            s = sg if s is None else s + sg
        m_prev = m_scr[...]
        m_new = jnp.maximum(m_prev, jnp.max(s, axis=1, keepdims=True))
        alpha = jnp.exp(m_prev - m_new)
        p = jnp.exp(s - m_new[:, 0:1])
        l_new = alpha * l_scr[...] + jnp.sum(p, axis=1, keepdims=True)
        l_scr[...] = l_new
        m_scr[...] = m_new
        pb = p.astype(bf16)

        start_job(j + L, 1, 2)

        acc = acc_scr[...] * alpha[:, 0:1]
        for g in range(G):
            og = lax.dot_general(pb, kvbuf[slot, 1, g], NN, preferred_element_type=f32)
            acc = acc + jnp.where(grp == g, og, 0.0)
        acc_scr[...] = acc

        @pl.when(c == CS - 1)
        def _():
            pm_scr[w] = m_new
            pl_scr[w] = l_new
            pa_scr[w] = acc

        return carry

    def finish(br):
        for hk in range(B * HKV):
            places = _places(br, hk)
            ms = [pm_scr[w, REP * i:REP * (i + 1), :] for w, i in places]
            ls = [pl_scr[w, REP * i:REP * (i + 1), :] for w, i in places]
            accs = [pa_scr[w, REP * i:REP * (i + 1), :] for w, i in places]
            if len(places) == 1:
                o = accs[0] / ls[0][:, 0:1]
            else:
                m = ms[0]
                for mk in ms[1:]:
                    m = jnp.maximum(m, mk)
                ws = [jnp.exp(mk - m) for mk in ms]
                l = ws[0] * ls[0]
                a = ws[0][:, 0:1] * accs[0]
                for wk, lk, ak_ in zip(ws[1:], ls[1:], accs[1:]):
                    l = l + wk * lk
                    a = a + wk[:, 0:1] * ak_
                o = a / l[:, 0:1]
            o = o.astype(bf16).astype(f32)
            b, h0 = hk // HKV, (hk % HKV) * REP
            for r in range(REP):
                o_scr[br, b:b + 1, (h0 + r) * DH:(h0 + r + 1) * DH] = o[r:r + 1, :]

    lax.fori_loop(0, NA, job, 0)

    xx = make_x(1)
    for pc in range(QP):
        qproj(1, xx, pc)
    finish(0)

    lax.fori_loop(NA, NJ, job, 0)
    finish(1)

    obs = [o_scr[br].astype(bf16) for br in range(2)]
    for gi, (brs, r0, nr, c0, cw, si, then_issue) in enumerate(WO_GROUPS):
        if gi == 1:
            issue_wo(4)
        dst = wobuf.at[pl.ds(brs[0], len(brs)), :, pl.ds(r0, nr), pl.ds(c0, cw)]
        pltpu.make_async_copy(dst, dst, sem.at[si]).wait()
        if then_issue is not None:
            issue_wo(then_issue)
        for br in brs:
            w = wobuf[br, :, r0:r0 + nr, c0:c0 + cw].reshape(WG * nr, cw)
            pt = lax.dot_general(obs[br][:, c0:c0 + cw], w, NT, preferred_element_type=f32)
            if c0 > 0:
                pt = pt + pp_scr[:, 0:WG * nr]
            if c0 + cw < E:
                pp_scr[:, 0:WG * nr] = pt
            else:
                for g in range(WG):
                    f0 = br * D + g * WR + r0
                    outf_scr[:, f0:f0 + nr] = pt[:, g * nr:(g + 1) * nr]

    o_ref[...] = outf_scr[0:B, :].astype(o_ref.dtype)


@jax.jit
def pallas_concat_heads__gqa_block_cached__sliding_block_cached__decode_kernel(
    A_x: jax.Array,
    A_k_cache: jax.Array,
    A_v_cache: jax.Array,
    A_wq: jax.Array,
    A_wo: jax.Array,
    B_x: jax.Array,
    B_k_cache: jax.Array,
    B_v_cache: jax.Array,
    B_wq: jax.Array,
    B_wo: jax.Array,
):
    hbm = pl.BlockSpec(memory_space=pltpu.HBM)
    bf16, f32 = jnp.bfloat16, jnp.float32
    out = pl.pallas_call(
        _kernel,
        out_shape=jax.ShapeDtypeStruct((B, 2 * D), bf16),
        in_specs=[hbm] * 10,
        out_specs=pl.BlockSpec(memory_space=pltpu.VMEM),
        scratch_shapes=[
            pltpu.VMEM((NB, 2, G, CH, DH), bf16),
            pltpu.VMEM((2, WG, WR, E), bf16),
            pltpu.VMEM((2, WG, WR, E), bf16),
            pltpu.VMEM((2, B, D), bf16),
            pltpu.VMEM((NSA + NSB, HQ, DH), f32),
            pltpu.VMEM((2, 8, E), f32),
            pltpu.VMEM((HQ, 128), f32),
            pltpu.VMEM((HQ, 128), f32),
            pltpu.VMEM((HQ, DH), f32),
            pltpu.VMEM((NSA + NSB, HQ, 128), f32),
            pltpu.VMEM((NSA + NSB, HQ, 128), f32),
            pltpu.VMEM((NSA + NSB, HQ, DH), f32),
            pltpu.VMEM((8, 2 * D), f32),
            pltpu.VMEM((8, 128), f32),
            pltpu.SemaphoreType.DMA((NSEM,)),
        ],
        compiler_params=pltpu.CompilerParams(vmem_limit_bytes=64 * 1024 * 1024),
    )(A_x.reshape(B, D), B_x.reshape(B, D),
      A_k_cache.reshape(NBA, BLK, DH), A_v_cache.reshape(NBA, BLK, DH),
      A_wq.reshape(WG, WR, E), A_wo.T.reshape(WG, WR, E),
      B_k_cache.reshape(NBB, SK, DH), B_v_cache.reshape(NBB, SK, DH),
      B_wq.reshape(WG, WR, E), B_wo.T.reshape(WG, WR, E))
    return out.reshape(B, 1, 2 * D)
```
